```python
import os as _os
_os.environ.setdefault("JAX_PLATFORMS", "cpu")
import jax
import jax.numpy as jnp

def _softmax(x, axis=-1):
    return jax.nn.softmax(x, axis=axis)
def _gelu(x):
    return jax.nn.gelu(x, approximate=True)
def _silu(x):
    return jax.nn.silu(x)
def _sigmoid(x):
    return jax.nn.sigmoid(x)
def _layernorm(x, axis=-1, eps=1e-5):
    m = jnp.mean(x, axis=axis, keepdims=True)
    v = jnp.var(x, axis=axis, keepdims=True)
    return (x - m) / jnp.sqrt(v + eps)
def _scatter_add(tgt, idx, src, axis=0):
    return tgt.at[idx].add(src)
def _segment_sum(src, seg, n):
    return jax.ops.segment_sum(src, seg, n)
class _Rng:
    def __init__(self, key):
        self._k = key
    def _next(self):
        self._k, sub = jax.random.split(self._k)
        return sub
    def normal(self, shape):
        return jax.random.normal(self._next(), shape, dtype=jnp.bfloat16)
    def randint(self, lo, hi, shape):
        return jax.random.randint(self._next(), shape, lo, hi, dtype=jnp.int32)
    def uniform(self, shape, lo=0.0, hi=1.0):
        return jax.random.uniform(self._next(), shape, jnp.bfloat16, lo, hi)
    def permutation(self, n):
        return jax.random.permutation(self._next(), n)


kernel_name = 'gated_mix__softmax_full_mha__spectral_gfnet__prompt'

def setup_inputs():
    _rng = _Rng(jax.random.key(int.from_bytes(__import__("os").urandom(4), "little")))
    _w = (lambda a: (lambda t: t.astype(jnp.bfloat16) if jnp.issubdtype(t.dtype, jnp.floating) else t)(jnp.asarray(a)))
    def _A_setup():
        B, S, D = 1, 2048, 448
        return {
            "x": _w((lambda *s: _rng.normal(s) * 0.05)(B, S, D)),
            "wqkv": _w((lambda *s: _rng.normal(s) * 0.4)(D, 3 * D)),
            "wo": _w((lambda *s: _rng.normal(s) * 0.05)(D, D)),
        }
    _A_in = _A_setup()

    def _B_setup():
        B, S, D = 1, 2048, 448
        Df = D // 2 + 1
        return {
            "x": _w((lambda *s: _rng.normal(s) * 0.05)(B, S, D)),
            "w_r": _w((lambda *s: _rng.normal(s) * 1.6)(S, Df) * 0.02),
            "w_i": _w((lambda *s: _rng.normal(s) * 1.6)(S, Df) * 0.02),
        }
    _B_in = _B_setup()

    return {
        "A_x": _A_in["x"],
        "A_wqkv": _A_in["wqkv"],
        "A_wo": _A_in["wo"],
        "B_x": _B_in["x"],
        "B_w_r": _B_in["w_r"],
        "B_w_i": _B_in["w_i"],
        "gate_w": _w((lambda *s: _rng.normal(s) * 0.05)(448) * 16.0),
    }

def reference(A_x, A_wqkv, A_wo, B_x, B_w_r, B_w_i, gate_w):
    def _A_ref(x, wqkv, wo):
        B, S, D = x.shape
        H = 16; Dh = D // H
        qkv = (lambda x, *d: x.transpose(*d))((x @ wqkv).reshape(B, S, 3, H, Dh), 2, 0, 3, 1, 4)
        q, k, v = qkv[0], qkv[1], qkv[2]
        scale = Dh ** -0.5
        scores = jnp.einsum("bhqd,bhkd->bhqk", q, k) * scale
        p = _softmax(scores, axis=-1)
        o = jnp.einsum("bhqk,bhkd->bhqd", p, v)
        return (lambda x, *d: x.transpose(*d))(o, 0, 2, 1, 3).reshape(B, S, D) @ wo

    def _B_ref(x, w_r, w_i):
        B, S, D = x.shape
        X = (lambda x, axes=(-2,-1): jnp.fft.rfft2(x.astype(jnp.float32), axes=axes))(x, axes=(-2, -1))
        W = w_r + 1j * w_i
        X = X * W
        y = (lambda x, s, axes=(-2,-1): jnp.fft.irfft2(x, s=s, axes=axes).astype(jnp.bfloat16))(X, (S, D), axes=(-2, -1))
        return y

    x = A_x
    g = _sigmoid((x * gate_w).sum(-1, keepdims=True))
    a = _A_ref(x, A_wqkv, A_wo)
    b = _B_ref(x, B_w_r, B_w_i)
    return g * a + (1 - g) * b
```

```python
import math

import numpy as np
import jax
import jax.numpy as jnp
from jax import lax
import jax.experimental.pallas as pl
import jax.experimental.pallas.tpu as pltpu

S = 2048
D = 448
H = 16
DH = 28
DF = D // 2 + 1
FP = 232
N1 = 16
N2 = 128
TQ = 512
NQ = S // TQ
F32 = jnp.float32
BF16 = jnp.bfloat16
SAFE_LOG2 = 60.0
GPI = 2
CB = D // 4
R1, R2, R3, R0 = 0, 56, 112, 168


def _consts():
    b = np.arange(CB)[None, :]

    def cs(f, n):
        f = np.concatenate([f, np.zeros(n - len(f), np.int64)])[:, None]
        ang = 2.0 * np.pi * ((f * b) % D) / D
        return np.cos(ang), np.sin(ang)
    f0 = np.arange(0, DF, 4)
    f1 = np.arange(1, DF, 4)
    f2 = np.arange(2, DF, 4)
    f3 = np.arange(3, DF, 4)
    c0, s0 = cs(f0, 64)
    c0[57:] = 0.0
    s0[57:] = 0.0
    c1, s1 = cs(f1, 56)
    c2, s2_ = cs(f2, 56)
    c3, s3 = cs(f3, 56)
    lp = np.concatenate([c0, -s0], axis=0)
    lm = np.concatenate([c2, -s2_], axis=0)
    lu = np.concatenate([c1, c3, -s1, -s3], axis=0)
    lv = np.concatenate([-s1, s3, -c1, c3], axis=0)
    fwd = np.concatenate([lp, lm, lu, lv], axis=0)

    def wgt(f, n):
        w = np.where((f == 0) | (f == DF - 1), 1.0, 2.0) / (S * D)
        return np.concatenate([w, np.zeros(n - len(f))])[None, :]
    w0, w1, w2, w3 = wgt(f0, 64), wgt(f1, 56), wgt(f2, 56), wgt(f3, 56)
    ip = np.concatenate([c0.T * w0, -s0.T * w0], axis=1)
    pad = np.zeros((CB, 16))
    im = np.concatenate([c2.T * w2, -s2_.T * w2, pad], axis=1)
    iu1 = np.concatenate([c1.T * w1, -s1.T * w1, pad], axis=1)
    iv1 = np.concatenate([s1.T * w1, c1.T * w1, pad], axis=1)
    iu3 = np.concatenate([c3.T * w3, -s3.T * w3, pad], axis=1)
    iv3 = np.concatenate([-s3.T * w3, -c3.T * w3, pad], axis=1)
    inv = np.concatenate([ip, im, iu1, iv1, iu3, iv3], axis=0)
    s2 = np.arange(N2)[:, None]
    k2 = np.arange(N2)[None, :]
    m = np.zeros((N1, 3, N2, N2))
    for k1 in range(N1):
        a = 2.0 * np.pi * ((s2 * (k1 + N1 * k2)) % S) / S
        mr, mi = np.cos(a), -np.sin(a)
        m[k1, 0] = mr
        m[k1, 1] = mi - mr
        m[k1, 2] = mr + mi
    return fwd, inv, m


def _cmul_const(re, im, c, s):
    eps = 1e-12
    if abs(s) < eps:
        if abs(c - 1) < eps:
            return re, im
        if abs(c + 1) < eps:
            return -re, -im
    if abs(c) < eps:
        if abs(s - 1) < eps:
            return -im, re
        if abs(s + 1) < eps:
            return im, -re
    if abs(abs(c) - abs(s)) < eps:
        if c * s > 0:
            return (re - im) * c, (re + im) * c
        return (re + im) * c, (im - re) * c
    return re * c - im * s, re * s + im * c


def _fft_list(xs, sign):
    n = len(xs)
    if n == 1:
        return xs
    ev = _fft_list(xs[0::2], sign)
    od = _fft_list(xs[1::2], sign)
    out = [None] * n
    for k in range(n // 2):
        ang = sign * 2.0 * math.pi * k / n
        tr, ti = _cmul_const(od[k][0], od[k][1], math.cos(ang), math.sin(ang))
        out[k] = (ev[k][0] + tr, ev[k][1] + ti)
        out[k + n // 2] = (ev[k][0] - tr, ev[k][1] - ti)
    return out


def _dft4(xs, sign):
    (ar, ai), (br, bi), (cr, ci), (dr, di) = xs
    sr, si = ar + cr, ai + ci
    tr, ti = ar - cr, ai - ci
    ur, ui = br + dr, bi + di
    vr, vi = br - dr, bi - di
    if sign < 0:
        wr, wi = vi, -vr
        return [(sr + ur, si + ui), (tr + vi, ti - vr), (sr - ur, si - ui), (tr - vi, ti + vr)]
    return [(sr + ur, si + ui), (tr - vi, ti + vr), (sr - ur, si - ui), (tr + vi, ti - vr)]


def _dft16_chunk(src, tmp, dst, r, sign, dst_rows):
    r8 = pl.multiple_of(r * 8, 8)
    re_rows, im_rows = pl.ds(r8, 8), pl.ds(FP + r8, 8)
    for a in range(4):
        ys = _dft4([(src[a + 4 * b, re_rows, :], src[a + 4 * b, im_rows, :]) for b in range(4)], sign)
        for c in range(4):
            ang = sign * 2.0 * math.pi * a * c / 16
            yr, yi = _cmul_const(ys[c][0], ys[c][1], math.cos(ang), math.sin(ang))
            tmp[a + 4 * c, re_rows, :] = yr
            tmp[a + 4 * c, im_rows, :] = yi
    dre, dim, dsum = dst_rows(r8)
    for c in range(4):
        ys = _dft4([(tmp[a + 4 * c, re_rows, :], tmp[a + 4 * c, im_rows, :]) for a in range(4)], sign)
        for d in range(4):
            dst[c + 4 * d, pl.ds(dre, 8), :] = ys[d][0].astype(dst.dtype)
            dst[c + 4 * d, pl.ds(dim, 8), :] = ys[d][1].astype(dst.dtype)
            if dsum is not None:
                dst[c + 4 * d, pl.ds(dsum, 8), :] = (ys[d][0] + ys[d][1]).astype(dst.dtype)


TB = 240


def _rows_same(r8):
    return TB + r8, 2 * TB + r8, r8


def _rows_class(r8):
    c2 = (r8 >= R2) & (r8 < R3)
    c3 = (r8 >= R3) & (r8 < R0)
    c0 = r8 >= R0
    dre = jnp.where(c0, r8 - R0, jnp.where(c3, r8 - R3 + 352, jnp.where(c2, r8 - R2 + 128, r8 + 240)))
    dim = dre + jnp.where(c0, 64, 56)
    return pl.multiple_of(dre, 8), pl.multiple_of(dim, 8), None


def _dot(a, b):
    return jnp.dot(a, b, preferred_element_type=F32)


def _dot_nt(a, b):
    return lax.dot_general(a, b, (((1,), (1,)), ((), ())), preferred_element_type=F32)


def _pad_heads(w):
    z = jnp.zeros((w.shape[0], 32 - DH), w.dtype)
    parts = []
    for h in range(H):
        parts += [w[:, h * DH:(h + 1) * DH], z]
    return jnp.concatenate(parts, axis=1)


def _kernel(xt_hbm, w_hbm, wo_hbm, wr_hbm, wi_hbm, gate_hbm, gt_hbm, git_hbm, m_hbm,
            o_hbm,
            xt_v, w_v, wo_v, wf_v, gate_v, gt_v, git_v, m_v, o_v, sems,
            k_s, qt_s, vt_s, ot_s, a_s, t_s, z_s, g_s, wn_s, wp_s, wot_s, wt_s, f_s):
    def cp(i, src, dst):
        return pltpu.make_async_copy(src, dst, sems.at[i])
    c_wq = cp(0, w_hbm.at[:, 0:512], w_v.at[:, 0:512])
    c_x = [cp(2 + i, xt_hbm.at[:, i * TQ:(i + 1) * TQ], xt_v.at[:, i * TQ:(i + 1) * TQ]) for i in range(NQ)]
    c_wkv = cp(12, w_hbm.at[:, 512:3 * D], w_v.at[:, 512:3 * D])
    c_gate = cp(1, gate_hbm, gate_v)
    c_gt = cp(6, gt_hbm, gt_v)
    c_wr = cp(7, wr_hbm, wf_v.at[0])
    c_wi = cp(8, wi_hbm, wf_v.at[1])
    c_m = cp(9, m_hbm, m_v)
    c_wo = cp(10, wo_hbm, wo_v)
    c_git = cp(11, git_hbm, git_v)
    for c in [c_wq] + c_x + [c_wkv, c_gate, c_gt]:
        c.start()

    qscale = (DH ** -0.5) * math.log2(math.e)
    stats = {}

    def upd(name, val):
        stats[name] = val if name not in stats else jnp.maximum(stats[name], val)

    def tilemax(a):
        return jnp.maximum(jnp.maximum(a[:, 0:128], a[:, 128:256]), jnp.maximum(a[:, 256:384], a[:, 384:512]))

    def dfwd(i):
        sl = slice(i * TQ, (i + 1) * TQ)
        xf = xt_v[:, sl].astype(F32)
        x0, x1, x2, x3 = (xf[a * CB:(a + 1) * CB] for a in range(4))
        e02, e13 = x0 + x2, x1 + x3
        rp = _dot(gt_v[0:128], (e02 + e13).astype(BF16))
        rm = _dot(gt_v[128:240], (e02 - e13).astype(BF16))
        ruv = (_dot(gt_v[240:464], (x0 - x2).astype(BF16)) + _dot(gt_v[464:688], (x1 - x3).astype(BF16)))
        for tt in range(TQ // N2):
            t = i * (TQ // N2) + tt
            ls = slice(tt * N2, (tt + 1) * N2)
            a_s[t, R0:R0 + 64, :] = rp[0:64, ls]
            a_s[t, FP + R0:FP + R0 + 64, :] = rp[64:128, ls]
            a_s[t, R2:R2 + 56, :] = rm[0:56, ls]
            a_s[t, FP + R2:FP + R2 + 56, :] = rm[56:112, ls]
            a_s[t, R1:R1 + 56, :] = ruv[0:56, ls]
            a_s[t, R3:R3 + 56, :] = ruv[56:112, ls]
            a_s[t, FP + R1:FP + R1 + 56, :] = ruv[112:168, ls]
            a_s[t, FP + R3:FP + R3 + 56, :] = ruv[168:224, ls]

    def proj(i, part):
        sl = slice(i * TQ, (i + 1) * TQ)
        r = _dot(wt_s[part] if part == 2 else wt_s[part, 0:D], xt_v[:, sl])
        if part == 0:
            qt = r[0:D] * qscale
            qt_s[:, sl] = qt.astype(BF16)
            upd("q", tilemax(jnp.abs(qt)))
        elif part == 1:
            kt = r[0:D]
            upd("k", tilemax(jnp.abs(kt)))
            z = jnp.zeros((16, TQ), BF16)
            for g in range(4):
                k_s[g, sl, :] = jnp.concatenate([kt[g * 112:(g + 1) * 112].astype(BF16), z], axis=0).T
        else:
            vt = r[0:D]
            g_s[:, sl] = jax.nn.sigmoid(r[D:D + 1])
            upd("v", jnp.max(tilemax(jnp.abs(vt)), axis=0, keepdims=True))
            tail = jnp.where(lax.broadcasted_iota(jnp.int32, (4, TQ), 0) == 0, 1.0, 0.0).astype(F32)
            parts = []
            for h in range(H):
                parts += [vt[h * DH:(h + 1) * DH], tail]
            vt_s[:, sl] = jnp.concatenate(parts, axis=0).astype(BF16)

    def wperm(c):
        wn_s[0] = pltpu.bitcast(wf_v[c, 0:128, :].T, jnp.uint32)
        u = pltpu.bitcast(wf_v[c, 128:DF, :].T, jnp.uint32)
        wn_s[1] = jnp.concatenate([u, jnp.zeros((S // 2, 256 - DF), jnp.uint32)], axis=1)
        for m in range(N1 // 2):
            for hf in range(2):
                wp_s[c, m, hf * 128:(hf + 1) * 128, :] = wn_s[hf, pl.ds(m, N2, stride=N1 // 2), :].T

    def smid(m, par):
        k1 = 2 * m + par
        ma = m_v[k1, 0]
        mb = m_v[k1, 1]
        mc = m_v[k1, 2]
        p1 = _dot(t_s[k1, 0:FP, :], ma)
        p2 = _dot(t_s[k1, TB:TB + FP, :], mb)
        p3 = _dot(t_s[k1, 2 * TB:2 * TB + FP, :], mc)
        xr = p1 - p3
        xi = p1 + p2

        def filt(c):
            u = jnp.concatenate(
                [wp_s[c, m, pl.ds(1, 56, stride=4), :], wp_s[c, m, pl.ds(2, 56, stride=4), :],
                 wp_s[c, m, pl.ds(3, 56, stride=4), :], wp_s[c, m, pl.ds(0, 64, stride=4), :]], axis=0)
            u = (u << 16) if par == 0 else (u & jnp.uint32(0xFFFF0000))
            return pltpu.bitcast(u, F32)
        wr, wi = filt(0), filt(1)
        yr = xr * wr - xi * wi
        yi = xr * wi + xi * wr
        q1 = _dot_nt((yr + yi).astype(BF16), ma)
        q2 = _dot_nt(yi.astype(BF16), mb)
        q3 = _dot_nt(yr.astype(BF16), mc)
        a_s[k1, 0:FP, :] = q1 + q2
        a_s[k1, FP:2 * FP, :] = q1 - q3

    NCH = FP // 8

    def dft_chunks(first, n, fwd):
        for j in range(n):
            r = jnp.minimum(first + j, NCH - 1)
            if fwd:
                _dft16_chunk(a_s, f_s, t_s, r, -1, _rows_same)
            else:
                _dft16_chunk(a_s, f_s, z_s, r, +1, _rows_class)

    c_wq.wait()
    wt_s[0, 0:D, :] = w_v[:, 0:D].T
    for i in range(NQ - 1):
        c_x[i].wait()
        proj(i, 0)
    c_x[NQ - 1].wait()
    c_wkv.wait()
    c_gate.wait()
    c_gt.wait()
    for c in [c_wo, c_wr, c_wi, c_m, c_git]:
        c.start()
    wt_s[1, 0:D, :] = w_v[:, D:2 * D].T
    wt_s[2, 0:D, :] = w_v[:, 2 * D:3 * D].T
    grow = lax.broadcasted_iota(jnp.int32, (16, D), 0)
    wt_s[2, D:D + 16, :] = jnp.where(grow == 0, jnp.broadcast_to(gate_v[...].reshape(1, D).astype(F32), (16, D)),
                                     0.0).astype(BF16)
    proj(NQ - 1, 0)
    for i in range(NQ):
        proj(i, 1)
    proj(0, 2)
    proj(1, 2)
    c_wo.wait()
    wot_s[...] = _pad_heads(wo_v[...].T)
    proj(2, 2)
    proj(3, 2)
    for i in range(NQ):
        dfwd(i)

    prod = (jnp.max(stats["q"], axis=1, keepdims=True) * jnp.max(stats["k"], axis=1, keepdims=True))
    prod = jnp.broadcast_to(prod, (D, 128))
    hr = lax.broadcasted_iota(jnp.int32, (D, 128), 0)
    hc = lax.broadcasted_iota(jnp.int32, (D, 128), 1) * DH
    hsel = (hr >= hc) & (hr < hc + DH)
    bound = jnp.max(jnp.sum(jnp.where(hsel, prod, 0.0), axis=0, keepdims=True))
    vtop = jnp.max(stats["v"])
    safe = (bound <= SAFE_LOG2) & (vtop <= 2.0 ** 40) & (vtop >= 2.0 ** -40)
    c_wr.wait()
    c_wi.wait()
    c_m.wait()
    c_git.wait()

    def head_weights(g, j, q0, tq):
        qg = qt_s[pl.ds(pl.multiple_of(g * 112, 16), 112), pl.ds(q0, tq)]
        w_all = pltpu.bitcast(jnp.concatenate([qg, jnp.zeros((16, tq), BF16)], axis=0), jnp.uint32)
        rows = lax.broadcasted_iota(jnp.int32, (64, tq), 0)
        msk = (rows >= 14 * j) & (rows < 14 * j + 14)
        return pltpu.bitcast(jnp.where(msk, w_all, jnp.uint32(0)), BF16)

    def attn_block(it):
        npq = 4 // GPI
        q0 = pl.multiple_of((it // npq) * TQ, TQ)
        for gg in range(GPI):
            g = (it % npq) * GPI + gg
            kg = k_s[g]
            for j in range(4):
                p = jnp.exp2(_dot(kg, head_weights(g, j, q0, TQ))).astype(BF16)
                h0 = pl.multiple_of((g * 4 + j) * 32, 32)
                acc = _dot(vt_s[pl.ds(h0, 32), :], p)
                ot_s[pl.ds(h0, 32), pl.ds(q0, TQ)] = (acc * (1.0 / acc[28:29, :])).astype(BF16)

    nit = NQ * 4 // GPI
    na = nit // 4
    nb = nit // 2
    per = -(-NCH // na)

    def body_a(it, carry):
        for cc in range(2 // na):
            wperm(it * (2 // na) + cc)
        dft_chunks(it * per, per, True)
        attn_block(it)
        return carry

    def body_b(it, carry):
        for kk in range(N1 // nb // 2):
            for par in range(2):
                smid((it - na) * (N1 // nb // 2) + kk, par)
        attn_block(it)
        return carry

    def body_c(it, carry):
        dft_chunks((it - na - nb) * per, per, False)
        attn_block(it)
        return carry

    def slow_unit(it, carry):
        tq = 128
        h = it // (S // tq)
        q0 = pl.multiple_of((it % (S // tq)) * tq, tq)
        g = h // 4
        s = _dot(k_s[g], head_weights(g, h % 4, q0, tq))
        p = jnp.exp2(s - jnp.max(s, axis=0, keepdims=True)).astype(BF16)
        h0 = pl.multiple_of(h * 32, 32)
        acc = _dot(vt_s[pl.ds(h0, 32), :], p)
        ot_s[pl.ds(h0, 32), pl.ds(q0, tq)] = (acc * (1.0 / acc[28:29, :])).astype(BF16)
        return carry

    def loop(n, f):
        def b(i, c):
            f(i)
            return c
        lax.fori_loop(0, n, b, 0)

    @pl.when(safe)
    def _():
        with jax.named_scope("loopA"):
            lax.fori_loop(0, na, body_a, 0)
        with jax.named_scope("loopB"):
            lax.fori_loop(na, na + nb, body_b, 0)
        with jax.named_scope("loopC"):
            lax.fori_loop(na + nb, nit, body_c, 0)

    @pl.when(jnp.logical_not(safe))
    def _():
        loop(2, wperm)
        loop(NCH, lambda r: _dft16_chunk(a_s, f_s, t_s, r, -1, _rows_same))
        loop(N1 // 2, lambda m: (smid(m, 0), smid(m, 1)))
        loop(NCH, lambda r: _dft16_chunk(a_s, f_s, z_s, r, +1, _rows_class))
        lax.fori_loop(0, H * (S // 128), slow_unit, 0)

    outs = []
    for qi in range(NQ):
        sl = slice(qi * TQ, (qi + 1) * TQ)
        at = _dot(wot_s[...], ot_s[:, sl])

        def zblk(r, n):
            return jnp.concatenate(
                [z_s[t, r:r + n, :] for t in range(qi * (TQ // N2), (qi + 1) * (TQ // N2))], axis=1)
        pp = _dot(git_v[0:112, :], zblk(0, 128))
        mm = _dot(git_v[112:224, 0:112], zblk(128, 112))
        uv = _dot(git_v[224:448, 0:112], zblk(240, 112)) + _dot(git_v[448:672, 0:112], zblk(352, 112))
        uu, vv = uv[0:112], uv[112:224]
        pms, pmd = pp + mm, pp - mm
        bt = jnp.concatenate([pms + uu, pmd - vv, pms - uu, pmd + vv], axis=0)
        g = g_s[:, sl]
        o_v[:, sl] = (g * at + (1.0 - g) * bt).astype(BF16)
        c = cp(13 + qi, o_v.at[:, sl], o_hbm.at[:, sl])
        c.start()
        outs.append(c)
    for c in outs:
        c.wait()


@jax.jit
def pallas_gated_mix__softmax_full_mha__spectral_gfnet__prompt_kernel(
    A_x, A_wqkv, A_wo, B_x, B_w_r, B_w_i, gate_w):
    del B_x
    xt = A_x.reshape(S, D).T
    gt, git, m = _consts()
    gt = jnp.asarray(gt, BF16)
    git = jnp.asarray(git, BF16)
    m = jnp.asarray(m, BF16)
    any_spec = pl.BlockSpec(memory_space=pl.ANY)
    out = pl.pallas_call(
        _kernel,
        out_shape=jax.ShapeDtypeStruct((D, S), BF16),
        in_specs=[any_spec] * 9,
        out_specs=any_spec,
        scratch_shapes=[
            pltpu.VMEM((D, S), BF16),
            pltpu.VMEM((D, 3 * D), BF16),
            pltpu.VMEM((D, D), BF16),
            pltpu.VMEM((2, DF, S), BF16),
            pltpu.VMEM((D,), BF16),
            pltpu.VMEM((688, CB), BF16),
            pltpu.VMEM((672, 128), BF16),
            pltpu.VMEM((N1, 3, N2, N2), BF16),
            pltpu.VMEM((D, S), BF16),
            pltpu.SemaphoreType.DMA((20,)),
            pltpu.VMEM((4, S, 128), BF16),
            pltpu.VMEM((D, S), BF16),
            pltpu.VMEM((512, S), BF16),
            pltpu.VMEM((512, S), BF16),
            pltpu.VMEM((N1, 2 * FP, N2), F32),
            pltpu.VMEM((N1, 3 * TB, N2), BF16),
            pltpu.VMEM((N1, 2 * FP, N2), BF16),
            pltpu.VMEM((1, S), F32),
            pltpu.VMEM((2, S // 2, 128), jnp.uint32),
            pltpu.VMEM((2, N1 // 2, 256, N2), jnp.uint32),
            pltpu.VMEM((D, 512), BF16),
            pltpu.VMEM((3, D + 16, D), BF16),
            pltpu.VMEM((N1, 2 * FP, N2), F32),
        ],
        compiler_params=pltpu.CompilerParams(vmem_limit_bytes=100 * 1024 * 1024),
    )(xt, A_wqkv, A_wo, B_w_r.T, B_w_i.T, gate_w, gt, git, m)
    return out.T.reshape(1, S, D)
```

```python
import math

import numpy as np
import jax
import jax.numpy as jnp
from jax import lax
import jax.experimental.pallas as pl
import jax.experimental.pallas.tpu as pltpu

S = 2048
D = 448
H = 16
DH = 28
DF = D // 2 + 1
FP = 232
N1 = 16
N2 = 128
TQ = 512
NQ = S // TQ
RSQRT2 = math.sqrt(0.5)
F32 = jnp.float32
BF16 = jnp.bfloat16
SAFE_LOG2 = 60.0
GPI = 2
CB = D // 8
R1, R2, R3, R0 = 0, 56, 112, 168


def _consts():
    cls = {r: np.arange(r, DF, 8) for r in range(8)}
    b = np.arange(CB)[None, :]
    zz = np.zeros

    def cs(f):
        ang = 2.0 * np.pi * ((f[:, None] * b) % D) / D
        return np.cos(ang), np.sin(ang)

    def wgt(f):
        return (np.where((f == 0) | (f == DF - 1), 1.0, 2.0) / (S * D))[None, :]
    c0, s0 = cs(cls[0])
    c4, s4 = cs(cls[4])
    re0 = np.concatenate([np.concatenate([c0, zz((29, CB))], 1), np.concatenate([zz((28, CB)), c4], 1),
                          zz((7, 2 * CB))], 0)
    im0 = np.concatenate([np.concatenate([-s0, zz((29, CB))], 1), np.concatenate([zz((28, CB)), -s4], 1),
                          zz((7, 2 * CB))], 0)
    fblocks = [np.concatenate([re0, im0], 0)]
    w0, w4 = wgt(cls[0]), wgt(cls[4])
    r0 = np.concatenate([c0.T * w0, zz((CB, 35)), -s0.T * w0, zz((CB, 35))], 1)
    r4 = np.concatenate([zz((CB, 29)), c4.T * w4, zz((CB, 36)), -s4.T * w4, zz((CB, 7))], 1)
    iblocks = [np.concatenate([r0, r4], 0)]
    for r in (1, 2, 3):
        ca, sa = cs(cls[r])
        cb, sb = cs(cls[8 - r])
        sg = -1.0 if r < 3 else 1.0
        re = np.concatenate([np.concatenate([ca, sg * sa], 1), np.concatenate([cb, -sg * sb], 1)], 0)
        im = np.concatenate([np.concatenate([-sa, sg * ca], 1), np.concatenate([-sb, -sg * cb], 1)], 0)
        fblocks.append(np.concatenate([re, im], 0))
        wa, wb = wgt(cls[r]), wgt(cls[8 - r])
        gre = np.concatenate([ca.T * wa, cb.T * wb, -sa.T * wa, -sb.T * wb], 1)
        gim = np.concatenate([sa.T * wa, -sb.T * wb, ca.T * wa, -cb.T * wb], 1)
        iblocks.append(np.concatenate([np.concatenate([gre, gim], 0), zz((2 * CB, 16))], 1))
    fwd = np.concatenate(fblocks, 0)
    inv = np.concatenate(iblocks, 0)
    s2 = np.arange(N2)[:, None]
    k2 = np.arange(N2)[None, :]
    m = np.zeros((N1, 6, N2, N2))
    for k1 in range(N1):
        a = 2.0 * np.pi * ((s2 * (k1 + N1 * k2)) % S) / S
        mr, mi = np.cos(a), -np.sin(a)
        m[k1, 0] = mr
        m[k1, 1] = mi - mr
        m[k1, 2] = mr + mi
        m[k1, 3] = mr.T
        m[k1, 4] = (mi - mr).T
        m[k1, 5] = (mr + mi).T
    return fwd, inv, m


def _cmul_const(re, im, c, s):
    eps = 1e-12
    if abs(s) < eps:
        if abs(c - 1) < eps:
            return re, im
        if abs(c + 1) < eps:
            return -re, -im
    if abs(c) < eps:
        if abs(s - 1) < eps:
            return -im, re
        if abs(s + 1) < eps:
            return im, -re
    if abs(abs(c) - abs(s)) < eps:
        if c * s > 0:
            return (re - im) * c, (re + im) * c
        return (re + im) * c, (im - re) * c
    return re * c - im * s, re * s + im * c


def _fft_list(xs, sign):
    n = len(xs)
    if n == 1:
        return xs
    ev = _fft_list(xs[0::2], sign)
    od = _fft_list(xs[1::2], sign)
    out = [None] * n
    for k in range(n // 2):
        ang = sign * 2.0 * math.pi * k / n
        tr, ti = _cmul_const(od[k][0], od[k][1], math.cos(ang), math.sin(ang))
        out[k] = (ev[k][0] + tr, ev[k][1] + ti)
        out[k + n // 2] = (ev[k][0] - tr, ev[k][1] - ti)
    return out


def _dft4(xs, sign):
    (ar, ai), (br, bi), (cr, ci), (dr, di) = xs
    sr, si = ar + cr, ai + ci
    tr, ti = ar - cr, ai - ci
    ur, ui = br + dr, bi + di
    vr, vi = br - dr, bi - di
    if sign < 0:
        wr, wi = vi, -vr
        return [(sr + ur, si + ui), (tr + vi, ti - vr), (sr - ur, si - ui), (tr - vi, ti + vr)]
    return [(sr + ur, si + ui), (tr - vi, ti + vr), (sr - ur, si - ui), (tr + vi, ti - vr)]


def _dft16_chunk(src, tmp, dst, r, sign, dst_rows):
    r8 = pl.multiple_of(r * 8, 8)
    re_rows, im_rows = pl.ds(r8, 8), pl.ds(FP + r8, 8)
    for a in range(4):
        ys = _dft4([(src[a + 4 * b, re_rows, :], src[a + 4 * b, im_rows, :]) for b in range(4)], sign)
        for c in range(4):
            ang = sign * 2.0 * math.pi * a * c / 16
            yr, yi = _cmul_const(ys[c][0], ys[c][1], math.cos(ang), math.sin(ang))
            tmp[a + 4 * c, re_rows, :] = yr
            tmp[a + 4 * c, im_rows, :] = yi
    dre, dim, dsum = dst_rows(r8)
    for c in range(4):
        ys = _dft4([(tmp[a + 4 * c, re_rows, :], tmp[a + 4 * c, im_rows, :]) for a in range(4)], sign)
        for d in range(4):
            dst[c + 4 * d, pl.ds(dre, 8), :] = ys[d][0].astype(dst.dtype)
            dst[c + 4 * d, pl.ds(dim, 8), :] = ys[d][1].astype(dst.dtype)
            if dsum is not None:
                dst[c + 4 * d, pl.ds(dsum, 8), :] = (ys[d][0] + ys[d][1]).astype(dst.dtype)


TB = 240


def _rows_same(r8):
    return TB + r8, 2 * TB + r8, r8


def _rows_class(r8):
    c2 = (r8 >= R2) & (r8 < R3)
    c3 = (r8 >= R3) & (r8 < R0)
    c0 = r8 >= R0
    dre = jnp.where(c0, r8 - R0, jnp.where(c3, r8 - R3 + 352, jnp.where(c2, r8 - R2 + 240, r8 + 128)))
    dim = dre + jnp.where(c0, 64, 56)
    return pl.multiple_of(dre, 8), pl.multiple_of(dim, 8), None


def _dot(a, b):
    return jnp.dot(a, b, preferred_element_type=F32)


def _dot_nt(a, b):
    return lax.dot_general(a, b, (((1,), (1,)), ((), ())), preferred_element_type=F32)


def _pad_heads(w):
    z = jnp.zeros((w.shape[0], 32 - DH), w.dtype)
    parts = []
    for h in range(H):
        parts += [w[:, h * DH:(h + 1) * DH], z]
    return jnp.concatenate(parts, axis=1)


def _kernel(xt_hbm, w_hbm, wo_hbm, wr_hbm, wi_hbm, gate_hbm, gt_hbm, git_hbm, m_hbm,
            o_hbm,
            xt_v, w_v, wo_v, wf_v, gate_v, gt_v, git_v, m_v, o_v, sems,
            k_s, qt_s, vt_s, ot_s, a_s, t_s, z_s, g_s, wn_s, wp_s, wot_s, wt_s, f_s):
    def cp(i, src, dst):
        return pltpu.make_async_copy(src, dst, sems.at[i])
    c_wq = cp(0, w_hbm.at[:, 0:512], w_v.at[:, 0:512])
    c_x = [cp(2 + i, xt_hbm.at[:, i * TQ:(i + 1) * TQ], xt_v.at[:, i * TQ:(i + 1) * TQ]) for i in range(NQ)]
    c_wkv = cp(12, w_hbm.at[:, 512:3 * D], w_v.at[:, 512:3 * D])
    c_gate = cp(1, gate_hbm, gate_v)
    c_gt = cp(6, gt_hbm, gt_v)
    c_wr = cp(7, wr_hbm, wf_v.at[0])
    c_wi = cp(8, wi_hbm, wf_v.at[1])
    c_m = cp(9, m_hbm, m_v)
    c_wo = cp(10, wo_hbm, wo_v)
    c_git = cp(11, git_hbm, git_v)
    for c in [c_gt, c_x[0], c_wq] + c_x[1:] + [c_wkv, c_gate]:
        c.start()

    qscale = (DH ** -0.5) * math.log2(math.e)
    stats = {}

    def upd(name, val):
        stats[name] = val if name not in stats else jnp.maximum(stats[name], val)

    def tilemax(a):
        return jnp.maximum(jnp.maximum(a[:, 0:128], a[:, 128:256]), jnp.maximum(a[:, 256:384], a[:, 384:512]))

    def dfwd(i):
        sl = slice(i * TQ, (i + 1) * TQ)
        xf = xt_v[:, sl].astype(F32)
        x = [xf[a * CB:(a + 1) * CB] for a in range(8)]
        s04, d04, s26, d26 = x[0] + x[4], x[0] - x[4], x[2] + x[6], x[2] - x[6]
        s15, d15, s37, d37 = x[1] + x[5], x[1] - x[5], x[3] + x[7], x[3] - x[7]
        e0, e1, o0, o1 = s04 + s26, s04 - s26, s15 + s37, s15 - s37
        p = (d15 - d37) * RSQRT2
        q = (d15 + d37) * RSQRT2

        def stack(u, v):
            return jnp.concatenate([u, v], axis=0).astype(BF16)
        r0 = _dot(gt_v[0:128], stack(e0 + o0, e0 - o0))
        r1 = _dot(gt_v[128:240], stack(d04 + p, d26 + q))
        r2 = _dot(gt_v[240:352], stack(e1, o1))
        r3 = _dot(gt_v[352:464], stack(d04 - p, d26 - q))
        for tt in range(TQ // N2):
            t = i * (TQ // N2) + tt
            ls = slice(tt * N2, (tt + 1) * N2)
            a_s[t, R0:R0 + 64, :] = r0[0:64, ls]
            a_s[t, FP + R0:FP + R0 + 64, :] = r0[64:128, ls]
            for rr, off in ((r1, R1), (r2, R2), (r3, R3)):
                a_s[t, off:off + 56, :] = rr[0:56, ls]
                a_s[t, FP + off:FP + off + 56, :] = rr[56:112, ls]

    def proj(i, part):
        sl = slice(i * TQ, (i + 1) * TQ)
        r = _dot(wt_s[part] if part == 2 else wt_s[part, 0:D], xt_v[:, sl])
        if part == 0:
            qt = r[0:D] * qscale
            qb = qt.astype(BF16)
            for tt in range(TQ // N2):
                qt_s[i * (TQ // N2) + tt] = qb[:, tt * N2:(tt + 1) * N2]
            upd("q", tilemax(jnp.abs(qt)))
        elif part == 1:
            kt = r[0:D]
            upd("k", tilemax(jnp.abs(kt)))
            z = jnp.zeros((16, TQ), BF16)
            for g in range(4):
                k_s[g, sl, :] = jnp.concatenate([kt[g * 112:(g + 1) * 112].astype(BF16), z], axis=0).T
        else:
            vt = r[0:D]
            g_s[:, sl] = jax.nn.sigmoid(r[D:D + 1])
            upd("v", jnp.max(tilemax(jnp.abs(vt)), axis=0, keepdims=True))
            tail = jnp.where(lax.broadcasted_iota(jnp.int32, (4, TQ), 0) == 0, 1.0, 0.0).astype(F32)
            parts = []
            for h in range(H):
                parts += [vt[h * DH:(h + 1) * DH], tail]
            vb = jnp.concatenate(parts, axis=0).astype(BF16)
            for tt in range(TQ // N2):
                vt_s[i * (TQ // N2) + tt] = vb[:, tt * N2:(tt + 1) * N2]

    def wperm(c):
        wn_s[0, 0:S // 2, :] = pltpu.bitcast(wf_v[c, 0:128, :].T, jnp.uint32)
        u = pltpu.bitcast(wf_v[c, 128:DF, :].T, jnp.uint32)
        wn_s[1, 0:S // 2, :] = jnp.concatenate([u, jnp.zeros((S // 2, 256 - DF), jnp.uint32)], axis=1)
        for m in range(N1 // 2):
            for hf in range(2):
                wp_s[c, m, hf * 128:(hf + 1) * 128, :] = wn_s[hf, pl.ds(m, N2, stride=N1 // 2), :].T

    def smid(m, par):
        k1 = 2 * m + par
        ma = m_v[k1, 0]
        mb = m_v[k1, 1]
        mc = m_v[k1, 2]
        p1 = _dot(t_s[k1, 0:FP, :], ma)
        p2 = _dot(t_s[k1, TB:TB + FP, :], mb)
        p3 = _dot(t_s[k1, 2 * TB:2 * TB + FP, :], mc)
        xr = p1 - p3
        xi = p1 + p2

        def filt(c):
            u = jnp.concatenate(
                [wp_s[c, m, pl.ds(f0, n, stride=8), :]
                 for f0, n in ((1, 28), (7, 28), (2, 28), (6, 28), (3, 28), (5, 28), (0, 29), (4, 28))]
                + [jnp.zeros((7, N2), jnp.uint32)], axis=0)
            u = (u << 16) if par == 0 else (u & jnp.uint32(0xFFFF0000))
            return pltpu.bitcast(u, F32)
        wr, wi = filt(0), filt(1)
        yr = xr * wr - xi * wi
        yi = xr * wi + xi * wr
        q1 = _dot((yr + yi).astype(BF16), m_v[k1, 3])
        q2 = _dot(yi.astype(BF16), m_v[k1, 4])
        q3 = _dot(yr.astype(BF16), m_v[k1, 5])
        a_s[k1, 0:FP, :] = q1 + q2
        a_s[k1, FP:2 * FP, :] = q1 - q3

    NCH = FP // 8

    def dft_chunks(first, n, fwd):
        for j in range(n):
            r = jnp.minimum(first + j, NCH - 1)
            if fwd:
                _dft16_chunk(a_s, f_s, t_s, r, -1, _rows_same)
            else:
                _dft16_chunk(a_s, f_s, z_s, r, +1, _rows_class)

    c_gt.wait()
    c_x[0].wait()
    dfwd(0)
    c_wq.wait()
    wt_s[0, 0:D, :] = w_v[:, 0:D].T
    proj(0, 0)
    c_x[1].wait()
    c_x[2].wait()
    proj(1, 0)
    dfwd(1)
    proj(2, 0)
    c_x[3].wait()
    c_wkv.wait()
    c_gate.wait()
    for c in [c_wo, c_wr, c_wi, c_m, c_git]:
        c.start()
    wt_s[1, 0:D, :] = w_v[:, D:2 * D].T
    wt_s[2, 0:D, :] = w_v[:, 2 * D:3 * D].T
    grow = lax.broadcasted_iota(jnp.int32, (16, D), 0)
    wt_s[2, D:D + 16, :] = jnp.where(grow == 0, jnp.broadcast_to(gate_v[...].reshape(1, D).astype(F32), (16, D)),
                                     0.0).astype(BF16)
    proj(3, 0)
    for i in range(NQ):
        proj(i, 1)
    proj(0, 2)
    proj(1, 2)
    c_wo.wait()
    wot_s[...] = _pad_heads(wo_v[...].T)
    proj(2, 2)
    proj(3, 2)
    dfwd(2)
    dfwd(3)

    prod = (jnp.max(stats["q"], axis=1, keepdims=True) * jnp.max(stats["k"], axis=1, keepdims=True))
    prod = jnp.broadcast_to(prod, (D, 128))
    hr = lax.broadcasted_iota(jnp.int32, (D, 128), 0)
    hc = lax.broadcasted_iota(jnp.int32, (D, 128), 1) * DH
    hsel = (hr >= hc) & (hr < hc + DH)
    bound = jnp.max(jnp.sum(jnp.where(hsel, prod, 0.0), axis=0, keepdims=True))
    vtop = jnp.max(stats["v"])
    safe = (bound <= SAFE_LOG2) & (vtop <= 2.0 ** 40) & (vtop >= 2.0 ** -40)
    c_wr.wait()
    c_wi.wait()
    c_m.wait()
    c_git.wait()

    def head_weights(g, j, q0, tq):
        t0 = q0 // N2
        qg = jnp.concatenate([qt_s[t0 + tt, pl.ds(pl.multiple_of(g * 112, 16), 112), :] for tt in range(tq // N2)], axis=1)
        w_all = pltpu.bitcast(jnp.concatenate([qg, jnp.zeros((16, tq), BF16)], axis=0), jnp.uint32)
        rows = lax.broadcasted_iota(jnp.int32, (64, tq), 0)
        msk = (rows >= 14 * j) & (rows < 14 * j + 14)
        return pltpu.bitcast(jnp.where(msk, w_all, jnp.uint32(0)), BF16)

    def vrows(h0):
        return jnp.concatenate([vt_s[t, pl.ds(h0, 32), :] for t in range(N1)], axis=1)

    def attn_block(it, gpi=GPI):
        npq = 4 // gpi
        q0 = pl.multiple_of((it // npq) * TQ, TQ)
        gq = g_s[:, pl.ds(q0, TQ)]
        for gg in range(gpi):
            g = (it % npq) * gpi + gg
            kg = k_s[g]
            for j in range(4):
                p = jnp.exp2(_dot(kg, head_weights(g, j, q0, TQ))).astype(BF16)
                h0 = pl.multiple_of((g * 4 + j) * 32, 32)
                acc = _dot(vrows(h0), p)
                ob = (acc * (gq / acc[28:29, :])).astype(BF16)
                for tt in range(TQ // N2):
                    ot_s[q0 // N2 + tt, pl.ds(h0, 32), :] = ob[:, tt * N2:(tt + 1) * N2]

    nit = NQ * 4 // GPI
    na = nit // 4
    nb = nit // 2
    per = -(-NCH // na)

    def body_a(it, carry):
        for cc in range(2 // na):
            wperm(it * (2 // na) + cc)
        dft_chunks(it * per, per, True)
        attn_block(it)
        return carry

    def body_b(it, carry):
        for kk in range(N1 // nb // 2):
            for par in range(2):
                smid((it - na) * (N1 // nb // 2) + kk, par)
        attn_block(it)
        return carry

    def body_c():
        dft_chunks(0, NCH, False)
        attn_block(NQ - 1, 4)

    def slow_unit(it, carry):
        tq = 128
        h = it // (S // tq)
        q0 = pl.multiple_of((it % (S // tq)) * tq, tq)
        g = h // 4
        s = _dot(k_s[g], head_weights(g, h % 4, q0, tq))
        p = jnp.exp2(s - jnp.max(s, axis=0, keepdims=True)).astype(BF16)
        h0 = pl.multiple_of(h * 32, 32)
        acc = _dot(vrows(h0), p)
        ot_s[q0 // N2, pl.ds(h0, 32), :] = (acc * (g_s[:, pl.ds(q0, tq)] / acc[28:29, :])).astype(BF16)
        return carry

    def loop(n, f):
        def b(i, c):
            f(i)
            return c
        lax.fori_loop(0, n, b, 0)

    @pl.when(safe)
    def _():
        lax.fori_loop(0, na, body_a, 0)
        lax.fori_loop(na, na + nb, body_b, 0)
        body_c()

    @pl.when(jnp.logical_not(safe))
    def _():
        loop(2, wperm)
        loop(NCH, lambda r: _dft16_chunk(a_s, f_s, t_s, r, -1, _rows_same))
        loop(N1 // 2, lambda m: (smid(m, 0), smid(m, 1)))
        loop(NCH, lambda r: _dft16_chunk(a_s, f_s, z_s, r, +1, _rows_class))
        lax.fori_loop(0, H * (S // 128), slow_unit, 0)

    chunks = [(0, 512), (512, 512), (1024, 512), (1536, 384), (1920, 128)]

    def out_mm(c0, n):
        sl = slice(c0, c0 + n)
        at = _dot(wot_s[...], jnp.concatenate([ot_s[t] for t in range(c0 // N2, (c0 + n) // N2)], axis=1))

        def zblk(r, m):
            return jnp.concatenate(
                [z_s[t, r:r + m, :] for t in range(c0 // N2, (c0 + n) // N2)], axis=1)
        rr = _dot(git_v[0:112, :], zblk(0, 128))
        gs = [_dot(git_v[112 * r:112 * (r + 1), 0:112], zblk(16 + 112 * r, 112)) for r in (1, 2, 3)]
        return at, rr, gs

    def out_fin(i, c0, n, at, rr, gs):
        sl = slice(c0, c0 + n)
        (g1, h1), (g2, h2), (g3, h3) = ((q[0:CB], q[CB:2 * CB]) for q in gs)
        ev, od = rr[0:CB] + rr[CB:2 * CB], rr[0:CB] - rr[CB:2 * CB]
        ep, em, om, op = ev + g2, ev - g2, od - h2, od + h2
        u, v = g1 + g3, h1 - h3
        dg, sh = g1 - g3, h1 + h3
        a1 = (dg - sh) * RSQRT2
        a3 = (dg + sh) * RSQRT2
        bt = jnp.concatenate([ep + u, om + a1, em - v, op - a3, ep - u, om - a1, em + v, op + a3], axis=0)
        g = g_s[:, sl]
        o_v[:, sl] = (at + (1.0 - g) * bt).astype(BF16)
        c = cp(13 + i, o_v.at[:, sl], o_hbm.at[:, sl])
        c.start()
        return c

    outs = []
    pend = out_mm(*chunks[0])
    for i, (c0, n) in enumerate(chunks):
        nxt = out_mm(*chunks[i + 1]) if i + 1 < len(chunks) else None
        outs.append(out_fin(i, c0, n, *pend))
        pend = nxt
    for c in outs:
        c.wait()


@jax.jit
def pallas_gated_mix__softmax_full_mha__spectral_gfnet__prompt_kernel(
    A_x, A_wqkv, A_wo, B_x, B_w_r, B_w_i, gate_w):
    del B_x
    xt = A_x.reshape(S, D).T
    gt, git, m = _consts()
    gt = jnp.asarray(gt, BF16)
    git = jnp.asarray(git, BF16)
    m = jnp.asarray(m, BF16)
    any_spec = pl.BlockSpec(memory_space=pl.ANY)
    out = pl.pallas_call(
        _kernel,
        out_shape=jax.ShapeDtypeStruct((D, S), BF16),
        in_specs=[any_spec] * 9,
        out_specs=any_spec,
        scratch_shapes=[
            pltpu.VMEM((D, S), BF16),
            pltpu.VMEM((D, 3 * D), BF16),
            pltpu.VMEM((D, D), BF16),
            pltpu.VMEM((2, DF, S), BF16),
            pltpu.VMEM((D,), BF16),
            pltpu.VMEM((464, 2 * CB), BF16),
            pltpu.VMEM((448, 128), BF16),
            pltpu.VMEM((N1, 6, N2, N2), BF16),
            pltpu.VMEM((D, S), BF16),
            pltpu.SemaphoreType.DMA((20,)),
            pltpu.VMEM((4, S, 128), BF16),
            pltpu.VMEM((N1, D, N2), BF16),
            pltpu.VMEM((N1, 512, N2), BF16),
            pltpu.VMEM((N1, 512, N2), BF16),
            pltpu.VMEM((N1, 2 * FP, N2), F32),
            pltpu.VMEM((N1, 3 * TB, N2), BF16),
            pltpu.VMEM((N1, 2 * FP, N2), BF16),
            pltpu.VMEM((1, S), F32),
            pltpu.VMEM((2, S // 2 + 8, 128), jnp.uint32),
            pltpu.VMEM((2, N1 // 2, 256, N2), jnp.uint32),
            pltpu.VMEM((D, 512), BF16),
            pltpu.VMEM((3, D + 16, D), BF16),
            pltpu.VMEM((N1, 2 * FP, N2), F32),
        ],
        compiler_params=pltpu.CompilerParams(vmem_limit_bytes=100 * 1024 * 1024),
    )(xt, A_wqkv, A_wo, B_w_r.T, B_w_i.T, gate_w, gt, git, m)
    return out.T.reshape(1, S, D)
```

```python
import math

import numpy as np
import jax
import jax.numpy as jnp
from jax import lax
import jax.experimental.pallas as pl
import jax.experimental.pallas.tpu as pltpu

S = 2048
D = 448
H = 16
DH = 28
DF = D // 2 + 1
FP = 232
N1 = 16
N2 = 128
TQ = 512
NQ = S // TQ
RSQRT2 = math.sqrt(0.5)
F32 = jnp.float32
BF16 = jnp.bfloat16
SAFE_LOG2 = 60.0
GPI = 2
CB = D // 8
R1, R2, R3, R0 = 0, 56, 112, 168


def _consts():
    cls = {r: np.arange(r, DF, 8) for r in range(8)}
    b = np.arange(CB)[None, :]
    zz = np.zeros

    def cs(f):
        ang = 2.0 * np.pi * ((f[:, None] * b) % D) / D
        return np.cos(ang), np.sin(ang)

    def wgt(f):
        return (np.where((f == 0) | (f == DF - 1), 1.0, 2.0) / (S * D))[None, :]
    c0, s0 = cs(cls[0])
    c4, s4 = cs(cls[4])
    re0 = np.concatenate([np.concatenate([c0, zz((29, CB))], 1), np.concatenate([zz((28, CB)), c4], 1),
                          zz((7, 2 * CB))], 0)
    im0 = np.concatenate([np.concatenate([-s0, zz((29, CB))], 1), np.concatenate([zz((28, CB)), -s4], 1),
                          zz((7, 2 * CB))], 0)
    fblocks = [np.concatenate([re0, im0], 0)]
    w0, w4 = wgt(cls[0]), wgt(cls[4])
    r0 = np.concatenate([c0.T * w0, zz((CB, 35)), -s0.T * w0, zz((CB, 35))], 1)
    r4 = np.concatenate([zz((CB, 29)), c4.T * w4, zz((CB, 36)), -s4.T * w4, zz((CB, 7))], 1)
    iblocks = [np.concatenate([r0, r4], 0)]
    for r in (1, 2, 3):
        ca, sa = cs(cls[r])
        cb, sb = cs(cls[8 - r])
        sg = -1.0 if r < 3 else 1.0
        re = np.concatenate([np.concatenate([ca, sg * sa], 1), np.concatenate([cb, -sg * sb], 1)], 0)
        im = np.concatenate([np.concatenate([-sa, sg * ca], 1), np.concatenate([-sb, -sg * cb], 1)], 0)
        fblocks.append(np.concatenate([re, im], 0))
        wa, wb = wgt(cls[r]), wgt(cls[8 - r])
        gre = np.concatenate([ca.T * wa, cb.T * wb, -sa.T * wa, -sb.T * wb], 1)
        gim = np.concatenate([sa.T * wa, -sb.T * wb, ca.T * wa, -cb.T * wb], 1)
        iblocks.append(np.concatenate([np.concatenate([gre, gim], 0), zz((2 * CB, 16))], 1))
    fwd = np.concatenate(fblocks, 0)
    inv = np.concatenate(iblocks, 0)
    s2 = np.arange(N2)[:, None]
    k2 = np.arange(N2)[None, :]
    m = np.zeros((N1, 6, N2, N2))
    for k1 in range(N1):
        a = 2.0 * np.pi * ((s2 * (k1 + N1 * k2)) % S) / S
        mr, mi = np.cos(a), -np.sin(a)
        m[k1, 0] = mr
        m[k1, 1] = mi - mr
        m[k1, 2] = mr + mi
        m[k1, 3] = mr.T
        m[k1, 4] = (mi - mr).T
        m[k1, 5] = (mr + mi).T
    return fwd, inv, m


def _cmul_const(re, im, c, s):
    eps = 1e-12
    if abs(s) < eps:
        if abs(c - 1) < eps:
            return re, im
        if abs(c + 1) < eps:
            return -re, -im
    if abs(c) < eps:
        if abs(s - 1) < eps:
            return -im, re
        if abs(s + 1) < eps:
            return im, -re
    if abs(abs(c) - abs(s)) < eps:
        if c * s > 0:
            return (re - im) * c, (re + im) * c
        return (re + im) * c, (im - re) * c
    return re * c - im * s, re * s + im * c


def _dft4(xs, sign):
    (ar, ai), (br, bi), (cr, ci), (dr, di) = xs
    sr, si = ar + cr, ai + ci
    tr, ti = ar - cr, ai - ci
    ur, ui = br + dr, bi + di
    vr, vi = br - dr, bi - di
    if sign < 0:
        return [(sr + ur, si + ui), (tr + vi, ti - vr), (sr - ur, si - ui), (tr - vi, ti + vr)]
    return [(sr + ur, si + ui), (tr - vi, ti + vr), (sr - ur, si - ui), (tr + vi, ti - vr)]


def _dft16_chunk(src, tmp, dst, r, sign, dst_rows):
    r8 = pl.multiple_of(r * 8, 8)
    re_rows, im_rows = pl.ds(r8, 8), pl.ds(FP + r8, 8)
    for a in range(4):
        ys = _dft4([(src[a + 4 * b, re_rows, :], src[a + 4 * b, im_rows, :]) for b in range(4)], sign)
        for c in range(4):
            ang = sign * 2.0 * math.pi * a * c / 16
            yr, yi = _cmul_const(ys[c][0], ys[c][1], math.cos(ang), math.sin(ang))
            tmp[a + 4 * c, re_rows, :] = yr
            tmp[a + 4 * c, im_rows, :] = yi
    dre, dim, dsum = dst_rows(r8)
    for c in range(4):
        ys = _dft4([(tmp[a + 4 * c, re_rows, :], tmp[a + 4 * c, im_rows, :]) for a in range(4)], sign)
        for d in range(4):
            dst[c + 4 * d, pl.ds(dre, 8), :] = ys[d][0].astype(dst.dtype)
            dst[c + 4 * d, pl.ds(dim, 8), :] = ys[d][1].astype(dst.dtype)
            if dsum is not None:
                dst[c + 4 * d, pl.ds(dsum, 8), :] = (ys[d][0] + ys[d][1]).astype(dst.dtype)


TB = 240


def _rows_same(r8):
    return TB + r8, 2 * TB + r8, r8


def _rows_class(r8):
    c2 = (r8 >= R2) & (r8 < R3)
    c3 = (r8 >= R3) & (r8 < R0)
    c0 = r8 >= R0
    dre = jnp.where(c0, r8 - R0, jnp.where(c3, r8 - R3 + 352, jnp.where(c2, r8 - R2 + 240, r8 + 128)))
    dim = dre + jnp.where(c0, 64, 56)
    return pl.multiple_of(dre, 8), pl.multiple_of(dim, 8), None


def _dot(a, b):
    return jnp.dot(a, b, preferred_element_type=F32)


def _pad_heads(w):
    z = jnp.zeros((w.shape[0], 32 - DH), w.dtype)
    parts = []
    for h in range(H):
        parts += [w[:, h * DH:(h + 1) * DH], z]
    return jnp.concatenate(parts, axis=1)


def _kernel(xt_hbm, w_hbm, wo_hbm, wr_hbm, wi_hbm, gate_hbm, gt_hbm, git_hbm, m_hbm,
            o_hbm,
            xt_v, w_v, wo_v, wf_v, gate_v, gt_v, git_v, m_v, o_v, sems,
            k_s, qt_s, vt_s, ot_s, a_s, t_s, z_s, g_s, wn_s, wp_s, wot_s, wt_s, f_s):
    def cp(i, src, dst):
        return pltpu.make_async_copy(src, dst, sems.at[i])
    c_wq = cp(0, w_hbm.at[:, 0:512], w_v.at[:, 0:512])
    c_x = [cp(2 + i, xt_hbm.at[:, i * TQ:(i + 1) * TQ], xt_v.at[:, i * TQ:(i + 1) * TQ]) for i in range(NQ)]
    c_wkv = cp(12, w_hbm.at[:, 512:3 * D], w_v.at[:, 512:3 * D])
    c_gate = cp(1, gate_hbm, gate_v)
    c_gt = cp(6, gt_hbm, gt_v)
    c_wr = cp(7, wr_hbm, wf_v.at[0])
    c_wi = cp(8, wi_hbm, wf_v.at[1])
    c_m = cp(9, m_hbm, m_v)
    c_wo = cp(10, wo_hbm, wo_v)
    c_git = cp(11, git_hbm, git_v)
    for c in [c_gt, c_x[0], c_wq] + c_x[1:] + [c_wkv, c_gate]:
        c.start()

    qscale = (DH ** -0.5) * math.log2(math.e)
    stats = {}

    def upd(name, val):
        stats[name] = val if name not in stats else jnp.maximum(stats[name], val)

    def tilemax(a):
        return jnp.maximum(jnp.maximum(a[:, 0:128], a[:, 128:256]), jnp.maximum(a[:, 256:384], a[:, 384:512]))

    def dfwd(i):
        sl = slice(i * TQ, (i + 1) * TQ)
        xf = xt_v[:, sl].astype(F32)
        x = [xf[a * CB:(a + 1) * CB] for a in range(8)]
        s04, d04, s26, d26 = x[0] + x[4], x[0] - x[4], x[2] + x[6], x[2] - x[6]
        s15, d15, s37, d37 = x[1] + x[5], x[1] - x[5], x[3] + x[7], x[3] - x[7]
        e0, e1, o0, o1 = s04 + s26, s04 - s26, s15 + s37, s15 - s37
        p = (d15 - d37) * RSQRT2
        q = (d15 + d37) * RSQRT2

        def stack(u, v):
            return jnp.concatenate([u, v], axis=0).astype(BF16)
        r0 = _dot(gt_v[0:128], stack(e0 + o0, e0 - o0))
        r1 = _dot(gt_v[128:240], stack(d04 + p, d26 + q))
        r2 = _dot(gt_v[240:352], stack(e1, o1))
        r3 = _dot(gt_v[352:464], stack(d04 - p, d26 - q))
        for tt in range(TQ // N2):
            t = i * (TQ // N2) + tt
            ls = slice(tt * N2, (tt + 1) * N2)
            a_s[t, R0:R0 + 64, :] = r0[0:64, ls]
            a_s[t, FP + R0:FP + R0 + 64, :] = r0[64:128, ls]
            for rr, off in ((r1, R1), (r2, R2), (r3, R3)):
                a_s[t, off:off + 56, :] = rr[0:56, ls]
                a_s[t, FP + off:FP + off + 56, :] = rr[56:112, ls]

    def proj(i, part):
        sl = slice(i * TQ, (i + 1) * TQ)
        r = _dot(wt_s[part] if part == 2 else wt_s[part, 0:D], xt_v[:, sl])
        if part == 0:
            qt = r[0:D] * qscale
            qb = qt.astype(BF16)
            for tt in range(TQ // N2):
                qt_s[i * (TQ // N2) + tt] = qb[:, tt * N2:(tt + 1) * N2]
            upd("q", tilemax(jnp.abs(qt)))
        elif part == 1:
            kt = r[0:D]
            upd("k", tilemax(jnp.abs(kt)))
            z = jnp.zeros((16, TQ), BF16)
            for g in range(4):
                k_s[g, sl, :] = jnp.concatenate([kt[g * 112:(g + 1) * 112].astype(BF16), z], axis=0).T
        else:
            vt = r[0:D]
            g_s[:, sl] = jax.nn.sigmoid(r[D:D + 1])
            upd("v", jnp.max(tilemax(jnp.abs(vt)), axis=0, keepdims=True))
            tail = jnp.where(lax.broadcasted_iota(jnp.int32, (4, TQ), 0) == 0, 1.0, 0.0).astype(F32)
            parts = []
            for h in range(H):
                parts += [vt[h * DH:(h + 1) * DH], tail]
            vb = jnp.concatenate(parts, axis=0).astype(BF16)
            for tt in range(TQ // N2):
                vt_s[i * (TQ // N2) + tt] = vb[:, tt * N2:(tt + 1) * N2]

    def wperm(c):
        wn_s[0, 0:S // 2, :] = pltpu.bitcast(wf_v[c, 0:128, :].T, jnp.uint32)
        u = pltpu.bitcast(wf_v[c, 128:DF, :].T, jnp.uint32)
        wn_s[1, 0:S // 2, :] = jnp.concatenate([u, jnp.zeros((S // 2, 256 - DF), jnp.uint32)], axis=1)
        for m in range(N1 // 2):
            for hf in range(2):
                wp_s[c, m, hf * 128:(hf + 1) * 128, :] = wn_s[hf, pl.ds(m, N2, stride=N1 // 2), :].T

    def smid(m, par):
        k1 = 2 * m + par
        p1 = _dot(t_s[k1, 0:FP, :], m_v[k1, 0])
        p2 = _dot(t_s[k1, TB:TB + FP, :], m_v[k1, 1])
        p3 = _dot(t_s[k1, 2 * TB:2 * TB + FP, :], m_v[k1, 2])
        xr = p1 - p3
        xi = p1 + p2

        def filt(c):
            u = jnp.concatenate(
                [wp_s[c, m, pl.ds(f0, n, stride=8), :]
                 for f0, n in ((1, 28), (7, 28), (2, 28), (6, 28), (3, 28), (5, 28), (0, 29), (4, 28))]
                + [jnp.zeros((7, N2), jnp.uint32)], axis=0)
            u = (u << 16) if par == 0 else (u & jnp.uint32(0xFFFF0000))
            return pltpu.bitcast(u, F32)
        wr, wi = filt(0), filt(1)
        yr = xr * wr - xi * wi
        yi = xr * wi + xi * wr
        q1 = _dot((yr + yi).astype(BF16), m_v[k1, 3])
        q2 = _dot(yi.astype(BF16), m_v[k1, 4])
        q3 = _dot(yr.astype(BF16), m_v[k1, 5])
        a_s[k1, 0:FP, :] = q1 + q2
        a_s[k1, FP:2 * FP, :] = q1 - q3

    NCH = FP // 8

    def dft_chunks(first, n, fwd):
        for j in range(n):
            r = jnp.minimum(first + j, NCH - 1)
            if fwd:
                _dft16_chunk(a_s, f_s, t_s, r, -1, _rows_same)
            else:
                _dft16_chunk(a_s, f_s, z_s, r, +1, _rows_class)

    c_gt.wait()
    c_x[0].wait()
    dfwd(0)
    c_wq.wait()
    wt_s[0, 0:D, :] = w_v[:, 0:D].T
    proj(0, 0)
    c_x[1].wait()
    c_x[2].wait()
    proj(1, 0)
    dfwd(1)
    proj(2, 0)
    c_x[3].wait()
    c_wkv.wait()
    c_gate.wait()
    for c in [c_wo, c_wr, c_wi, c_m, c_git]:
        c.start()
    wt_s[1, 0:D, :] = w_v[:, D:2 * D].T
    wt_s[2, 0:D, :] = w_v[:, 2 * D:3 * D].T
    grow = lax.broadcasted_iota(jnp.int32, (16, D), 0)
    wt_s[2, D:D + 16, :] = jnp.where(grow == 0, jnp.broadcast_to(gate_v[...].reshape(1, D).astype(F32), (16, D)),
                                     0.0).astype(BF16)
    proj(3, 0)
    for i in range(NQ):
        proj(i, 1)
    proj(0, 2)
    proj(1, 2)
    c_wo.wait()
    wot_s[...] = _pad_heads(wo_v[...].T)
    proj(2, 2)
    proj(3, 2)
    dfwd(2)
    dfwd(3)

    prod = (jnp.max(stats["q"], axis=1, keepdims=True) * jnp.max(stats["k"], axis=1, keepdims=True))
    prod = jnp.broadcast_to(prod, (D, 128))
    hr = lax.broadcasted_iota(jnp.int32, (D, 128), 0)
    hc = lax.broadcasted_iota(jnp.int32, (D, 128), 1) * DH
    hsel = (hr >= hc) & (hr < hc + DH)
    bound = jnp.max(jnp.sum(jnp.where(hsel, prod, 0.0), axis=0, keepdims=True))
    vtop = jnp.max(stats["v"])
    safe = (bound <= SAFE_LOG2) & (vtop <= 2.0 ** 40) & (vtop >= 2.0 ** -40)
    c_wr.wait()
    c_wi.wait()
    c_m.wait()
    c_git.wait()

    def head_weights(g, j, q0, tq):
        t0 = q0 // N2
        qg = jnp.concatenate([qt_s[t0 + tt, pl.ds(pl.multiple_of(g * 112, 16), 112), :] for tt in range(tq // N2)], axis=1)
        w_all = pltpu.bitcast(jnp.concatenate([qg, jnp.zeros((16, tq), BF16)], axis=0), jnp.uint32)
        rows = lax.broadcasted_iota(jnp.int32, (64, tq), 0)
        msk = (rows >= 14 * j) & (rows < 14 * j + 14)
        return pltpu.bitcast(jnp.where(msk, w_all, jnp.uint32(0)), BF16)

    def vrows(h0):
        return jnp.concatenate([vt_s[t, pl.ds(h0, 32), :] for t in range(N1)], axis=1)

    def attn_block(it, gpi=GPI):
        npq = 4 // gpi
        q0 = pl.multiple_of((it // npq) * TQ, TQ)
        gq = g_s[:, pl.ds(q0, TQ)]
        for gg in range(gpi):
            g = (it % npq) * gpi + gg
            kg = k_s[g]
            for j in range(4):
                p = jnp.exp2(_dot(kg, head_weights(g, j, q0, TQ))).astype(BF16)
                h0 = pl.multiple_of((g * 4 + j) * 32, 32)
                acc = _dot(vrows(h0), p)
                ob = (acc * (gq / acc[28:29, :])).astype(BF16)
                for tt in range(TQ // N2):
                    ot_s[q0 // N2 + tt, pl.ds(h0, 32), :] = ob[:, tt * N2:(tt + 1) * N2]

    nit = NQ * 4 // GPI
    na = nit // 4
    nb = nit // 2
    per = -(-NCH // na)

    def body_a(it, carry):
        for cc in range(2 // na):
            wperm(it * (2 // na) + cc)
        dft_chunks(it * per, per, True)
        attn_block(it)
        return carry

    def body_b(it, carry):
        for kk in range(N1 // nb // 2):
            for par in range(2):
                smid((it - na) * (N1 // nb // 2) + kk, par)
        attn_block(it)
        return carry

    def body_c():
        dft_chunks(0, NCH, False)
        attn_block(NQ - 1, 4)

    def slow_unit(it, carry):
        tq = 128
        h = it // (S // tq)
        q0 = pl.multiple_of((it % (S // tq)) * tq, tq)
        g = h // 4
        s = _dot(k_s[g], head_weights(g, h % 4, q0, tq))
        p = jnp.exp2(s - jnp.max(s, axis=0, keepdims=True)).astype(BF16)
        h0 = pl.multiple_of(h * 32, 32)
        acc = _dot(vrows(h0), p)
        ot_s[q0 // N2, pl.ds(h0, 32), :] = (acc * (g_s[:, pl.ds(q0, tq)] / acc[28:29, :])).astype(BF16)
        return carry

    def loop(n, f):
        def b(i, c):
            f(i)
            return c
        lax.fori_loop(0, n, b, 0)

    @pl.when(safe)
    def _():
        lax.fori_loop(0, na, body_a, 0)
        lax.fori_loop(na, na + nb, body_b, 0)
        body_c()

    @pl.when(jnp.logical_not(safe))
    def _():
        loop(2, wperm)
        loop(NCH, lambda r: _dft16_chunk(a_s, f_s, t_s, r, -1, _rows_same))
        loop(N1 // 2, lambda m: (smid(m, 0), smid(m, 1)))
        loop(NCH, lambda r: _dft16_chunk(a_s, f_s, z_s, r, +1, _rows_class))
        lax.fori_loop(0, H * (S // 128), slow_unit, 0)

    chunks = [(0, 512), (512, 512), (1024, 512), (1536, 384), (1920, 128)]

    def out_mm(c0, n):
        sl = slice(c0, c0 + n)
        at = _dot(wot_s[...], jnp.concatenate([ot_s[t] for t in range(c0 // N2, (c0 + n) // N2)], axis=1))

        def zblk(r, m):
            return jnp.concatenate(
                [z_s[t, r:r + m, :] for t in range(c0 // N2, (c0 + n) // N2)], axis=1)
        rr = _dot(git_v[0:112, :], zblk(0, 128))
        gs = [_dot(git_v[112 * r:112 * (r + 1), 0:112], zblk(16 + 112 * r, 112)) for r in (1, 2, 3)]
        return at, rr, gs

    def out_fin(i, c0, n, at, rr, gs):
        sl = slice(c0, c0 + n)
        (g1, h1), (g2, h2), (g3, h3) = ((q[0:CB], q[CB:2 * CB]) for q in gs)
        ev, od = rr[0:CB] + rr[CB:2 * CB], rr[0:CB] - rr[CB:2 * CB]
        ep, em, om, op = ev + g2, ev - g2, od - h2, od + h2
        u, v = g1 + g3, h1 - h3
        dg, sh = g1 - g3, h1 + h3
        a1 = (dg - sh) * RSQRT2
        a3 = (dg + sh) * RSQRT2
        bt = jnp.concatenate([ep + u, om + a1, em - v, op - a3, ep - u, om - a1, em + v, op + a3], axis=0)
        g = g_s[:, sl]
        o_v[:, sl] = (at + (1.0 - g) * bt).astype(BF16)
        c = cp(13 + i, o_v.at[:, sl], o_hbm.at[:, sl])
        c.start()
        return c

    outs = []
    pend = out_mm(*chunks[0])
    for i, (c0, n) in enumerate(chunks):
        nxt = out_mm(*chunks[i + 1]) if i + 1 < len(chunks) else None
        outs.append(out_fin(i, c0, n, *pend))
        pend = nxt
    for c in outs:
        c.wait()


@jax.jit
def pallas_gated_mix__softmax_full_mha__spectral_gfnet__prompt_kernel(
    A_x, A_wqkv, A_wo, B_x, B_w_r, B_w_i, gate_w):
    del B_x
    xt = A_x.reshape(S, D).T
    gt, git, m = _consts()
    gt = jnp.asarray(gt, BF16)
    git = jnp.asarray(git, BF16)
    m = jnp.asarray(m, BF16)
    any_spec = pl.BlockSpec(memory_space=pl.ANY)
    out = pl.pallas_call(
        _kernel,
        out_shape=jax.ShapeDtypeStruct((D, S), BF16),
        in_specs=[any_spec] * 9,
        out_specs=any_spec,
        scratch_shapes=[
            pltpu.VMEM((D, S), BF16),
            pltpu.VMEM((D, 3 * D), BF16),
            pltpu.VMEM((D, D), BF16),
            pltpu.VMEM((2, DF, S), BF16),
            pltpu.VMEM((D,), BF16),
            pltpu.VMEM((464, 2 * CB), BF16),
            pltpu.VMEM((448, 128), BF16),
            pltpu.VMEM((N1, 6, N2, N2), BF16),
            pltpu.VMEM((D, S), BF16),
            pltpu.SemaphoreType.DMA((20,)),
            pltpu.VMEM((4, S, 128), BF16),
            pltpu.VMEM((N1, D, N2), BF16),
            pltpu.VMEM((N1, 512, N2), BF16),
            pltpu.VMEM((N1, 512, N2), BF16),
            pltpu.VMEM((N1, 2 * FP, N2), F32),
            pltpu.VMEM((N1, 3 * TB, N2), BF16),
            pltpu.VMEM((N1, 2 * FP, N2), BF16),
            pltpu.VMEM((1, S), F32),
            pltpu.VMEM((2, S // 2 + 8, 128), jnp.uint32),
            pltpu.VMEM((2, N1 // 2, 256, N2), jnp.uint32),
            pltpu.VMEM((D, 512), BF16),
            pltpu.VMEM((3, D + 16, D), BF16),
            pltpu.VMEM((N1, 2 * FP, N2), F32),
        ],
        compiler_params=pltpu.CompilerParams(vmem_limit_bytes=100 * 1024 * 1024),
    )(xt, A_wqkv, A_wo, B_w_r.T, B_w_i.T, gate_w, gt, git, m)
    return out.T.reshape(1, S, D)
```

```python
import math

import numpy as np
import jax
import jax.numpy as jnp
from jax import lax
import jax.experimental.pallas as pl
import jax.experimental.pallas.tpu as pltpu

S = 2048
D = 448
H = 16
DH = 28
DF = D // 2 + 1
FP = 232
N1 = 16
N2 = 128
TQ = 512
NQ = S // TQ
RSQRT2 = math.sqrt(0.5)
F32 = jnp.float32
BF16 = jnp.bfloat16
SAFE_LOG2 = 60.0
CB = D // 8
R1, R2, R3, R0 = 0, 56, 112, 168


def _consts():
    cls = {r: np.arange(r, DF, 8) for r in range(8)}
    b = np.arange(CB)[None, :]
    zz = np.zeros

    def cs(f):
        ang = 2.0 * np.pi * ((f[:, None] * b) % D) / D
        return np.cos(ang), np.sin(ang)

    def wgt(f):
        return (np.where((f == 0) | (f == DF - 1), 1.0, 2.0) / (S * D))[None, :]
    c0, s0 = cs(cls[0])
    c4, s4 = cs(cls[4])
    re0 = np.concatenate([np.concatenate([c0, zz((29, CB))], 1), np.concatenate([zz((28, CB)), c4], 1),
                          zz((7, 2 * CB))], 0)
    im0 = np.concatenate([np.concatenate([-s0, zz((29, CB))], 1), np.concatenate([zz((28, CB)), -s4], 1),
                          zz((7, 2 * CB))], 0)
    fblocks = [np.concatenate([re0, im0], 0)]
    w0, w4 = wgt(cls[0]), wgt(cls[4])
    r0 = np.concatenate([c0.T * w0, zz((CB, 35)), -s0.T * w0, zz((CB, 35))], 1)
    r4 = np.concatenate([zz((CB, 29)), c4.T * w4, zz((CB, 36)), -s4.T * w4, zz((CB, 7))], 1)
    iblocks = [np.concatenate([r0, r4], 0)]
    for r in (1, 2, 3):
        ca, sa = cs(cls[r])
        cb, sb = cs(cls[8 - r])
        sg = -1.0 if r < 3 else 1.0
        re = np.concatenate([np.concatenate([ca, sg * sa], 1), np.concatenate([cb, -sg * sb], 1)], 0)
        im = np.concatenate([np.concatenate([-sa, sg * ca], 1), np.concatenate([-sb, -sg * cb], 1)], 0)
        fblocks.append(np.concatenate([re, im], 0))
        wa, wb = wgt(cls[r]), wgt(cls[8 - r])
        gre = np.concatenate([ca.T * wa, cb.T * wb, -sa.T * wa, -sb.T * wb], 1)
        gim = np.concatenate([sa.T * wa, -sb.T * wb, ca.T * wa, -cb.T * wb], 1)
        iblocks.append(np.concatenate([np.concatenate([gre, gim], 0), zz((2 * CB, 16))], 1))
    fwd = np.concatenate(fblocks, 0)
    inv = np.concatenate(iblocks, 0)
    s2 = np.arange(N2)[:, None]
    k2 = np.arange(N2)[None, :]
    m = np.zeros((N1, 6, N2, N2))
    for k1 in range(N1):
        a = 2.0 * np.pi * ((s2 * (k1 + N1 * k2)) % S) / S
        mr, mi = np.cos(a), -np.sin(a)
        m[k1, 0] = mr
        m[k1, 1] = mi - mr
        m[k1, 2] = mr + mi
        m[k1, 3] = mr.T
        m[k1, 4] = (mi - mr).T
        m[k1, 5] = (mr + mi).T
    return fwd, inv, m


def _cmul_const(re, im, c, s):
    eps = 1e-12
    if abs(s) < eps:
        if abs(c - 1) < eps:
            return re, im
        if abs(c + 1) < eps:
            return -re, -im
    if abs(c) < eps:
        if abs(s - 1) < eps:
            return -im, re
        if abs(s + 1) < eps:
            return im, -re
    if abs(abs(c) - abs(s)) < eps:
        if c * s > 0:
            return (re - im) * c, (re + im) * c
        return (re + im) * c, (im - re) * c
    return re * c - im * s, re * s + im * c


def _dft4(xs, sign):
    (ar, ai), (br, bi), (cr, ci), (dr, di) = xs
    sr, si = ar + cr, ai + ci
    tr, ti = ar - cr, ai - ci
    ur, ui = br + dr, bi + di
    vr, vi = br - dr, bi - di
    if sign < 0:
        return [(sr + ur, si + ui), (tr + vi, ti - vr), (sr - ur, si - ui), (tr - vi, ti + vr)]
    return [(sr + ur, si + ui), (tr - vi, ti + vr), (sr - ur, si - ui), (tr + vi, ti - vr)]


def _dft16_chunk(src, tmp, dst, r, sign, dst_rows):
    r8 = pl.multiple_of(r * 8, 8)
    re_rows, im_rows = pl.ds(r8, 8), pl.ds(FP + r8, 8)
    for a in range(4):
        ys = _dft4([(src[a + 4 * b, re_rows, :], src[a + 4 * b, im_rows, :]) for b in range(4)], sign)
        for c in range(4):
            ang = sign * 2.0 * math.pi * a * c / 16
            yr, yi = _cmul_const(ys[c][0], ys[c][1], math.cos(ang), math.sin(ang))
            tmp[a + 4 * c, re_rows, :] = yr
            tmp[a + 4 * c, im_rows, :] = yi
    dre, dim, dsum = dst_rows(r8)
    for c in range(4):
        ys = _dft4([(tmp[a + 4 * c, re_rows, :], tmp[a + 4 * c, im_rows, :]) for a in range(4)], sign)
        for d in range(4):
            dst[c + 4 * d, pl.ds(dre, 8), :] = ys[d][0].astype(dst.dtype)
            dst[c + 4 * d, pl.ds(dim, 8), :] = ys[d][1].astype(dst.dtype)
            if dsum is not None:
                dst[c + 4 * d, pl.ds(dsum, 8), :] = (ys[d][0] + ys[d][1]).astype(dst.dtype)


TB = 240


def _rows_same(r8):
    return TB + r8, 2 * TB + r8, r8


def _rows_class(r8):
    c2 = (r8 >= R2) & (r8 < R3)
    c3 = (r8 >= R3) & (r8 < R0)
    c0 = r8 >= R0
    dre = jnp.where(c0, r8 - R0, jnp.where(c3, r8 - R3 + 352, jnp.where(c2, r8 - R2 + 240, r8 + 128)))
    dim = dre + jnp.where(c0, 64, 56)
    return pl.multiple_of(dre, 8), pl.multiple_of(dim, 8), None


def _dot(a, b):
    return jnp.dot(a, b, preferred_element_type=F32)


def _pad_heads(w):
    z = jnp.zeros((w.shape[0], 32 - DH), w.dtype)
    parts = []
    for h in range(H):
        parts += [w[:, h * DH:(h + 1) * DH], z]
    return jnp.concatenate(parts, axis=1)


def _kernel(xt_hbm, w_hbm, wo_hbm, wr_hbm, wi_hbm, gate_hbm, gt_hbm, git_hbm, m_hbm,
            o_hbm,
            xt_v, w_v, wo_v, wf_v, gate_v, gt_v, git_v, m_v, o_v, sems,
            k_s, qt_s, vt_s, ot_s, a_s, t_s, z_s, g_s, wn_s, wp_s, wot_s, wt_s, f_s):
    def cp(i, src, dst):
        return pltpu.make_async_copy(src, dst, sems.at[i])
    c_wq = cp(0, w_hbm.at[:, 0:512], w_v.at[:, 0:512])
    c_x = [cp(2 + i, xt_hbm.at[:, i * TQ:(i + 1) * TQ], xt_v.at[:, i * TQ:(i + 1) * TQ]) for i in range(NQ)]
    c_wkv = cp(12, w_hbm.at[:, 512:3 * D], w_v.at[:, 512:3 * D])
    c_gate = cp(1, gate_hbm, gate_v)
    c_gt = cp(6, gt_hbm, gt_v)
    c_wr = cp(7, wr_hbm, wf_v.at[0])
    c_wi = cp(8, wi_hbm, wf_v.at[1])
    c_m = cp(9, m_hbm, m_v)
    c_wo = cp(10, wo_hbm, wo_v)
    c_git = cp(11, git_hbm, git_v)
    for c in [c_gt, c_x[0], c_wq] + c_x[1:] + [c_wkv, c_gate]:
        c.start()

    qscale = (DH ** -0.5) * math.log2(math.e)
    stats = {}

    def upd(name, val):
        stats[name] = val if name not in stats else jnp.maximum(stats[name], val)

    def tilemax(a):
        return jnp.maximum(jnp.maximum(a[:, 0:128], a[:, 128:256]), jnp.maximum(a[:, 256:384], a[:, 384:512]))

    def dfwd(i):
        sl = slice(i * TQ, (i + 1) * TQ)
        xf = xt_v[:, sl].astype(F32)
        x = [xf[a * CB:(a + 1) * CB] for a in range(8)]
        s04, d04, s26, d26 = x[0] + x[4], x[0] - x[4], x[2] + x[6], x[2] - x[6]
        s15, d15, s37, d37 = x[1] + x[5], x[1] - x[5], x[3] + x[7], x[3] - x[7]
        e0, e1, o0, o1 = s04 + s26, s04 - s26, s15 + s37, s15 - s37
        p = (d15 - d37) * RSQRT2
        q = (d15 + d37) * RSQRT2

        def stack(u, v):
            return jnp.concatenate([u, v], axis=0).astype(BF16)
        r0 = _dot(gt_v[0:128], stack(e0 + o0, e0 - o0))
        r1 = _dot(gt_v[128:240], stack(d04 + p, d26 + q))
        r2 = _dot(gt_v[240:352], stack(e1, o1))
        r3 = _dot(gt_v[352:464], stack(d04 - p, d26 - q))
        for tt in range(TQ // N2):
            t = i * (TQ // N2) + tt
            ls = slice(tt * N2, (tt + 1) * N2)
            a_s[t, R0:R0 + 64, :] = r0[0:64, ls]
            a_s[t, FP + R0:FP + R0 + 64, :] = r0[64:128, ls]
            for rr, off in ((r1, R1), (r2, R2), (r3, R3)):
                a_s[t, off:off + 56, :] = rr[0:56, ls]
                a_s[t, FP + off:FP + off + 56, :] = rr[56:112, ls]

    def proj(i, part):
        sl = slice(i * TQ, (i + 1) * TQ)
        r = _dot(wt_s[part] if part == 2 else wt_s[part, 0:D], xt_v[:, sl])
        if part == 0:
            qt = r[0:D] * qscale
            qb = qt.astype(BF16)
            for tt in range(TQ // N2):
                qt_s[i * (TQ // N2) + tt] = qb[:, tt * N2:(tt + 1) * N2]
            upd("q", tilemax(jnp.abs(qt)))
        elif part == 1:
            kt = r[0:D]
            upd("k", tilemax(jnp.abs(kt)))
            z = jnp.zeros((16, TQ), BF16)
            for g in range(4):
                k_s[g, sl, :] = jnp.concatenate([kt[g * 112:(g + 1) * 112].astype(BF16), z], axis=0).T
        else:
            vt = r[0:D]
            g_s[:, sl] = jax.nn.sigmoid(r[D:D + 1])
            upd("v", jnp.max(tilemax(jnp.abs(vt)), axis=0, keepdims=True))
            tail = jnp.where(lax.broadcasted_iota(jnp.int32, (4, TQ), 0) == 0, 1.0, 0.0).astype(F32)
            parts = []
            for h in range(H):
                parts += [vt[h * DH:(h + 1) * DH], tail]
            vb = jnp.concatenate(parts, axis=0).astype(BF16)
            for tt in range(TQ // N2):
                vt_s[i * (TQ // N2) + tt] = vb[:, tt * N2:(tt + 1) * N2]

    def wperm(c):
        wn_s[0, 0:S // 2, :] = pltpu.bitcast(wf_v[c, 0:128, :].T, jnp.uint32)
        u = pltpu.bitcast(wf_v[c, 128:DF, :].T, jnp.uint32)
        wn_s[1, 0:S // 2, :] = jnp.concatenate([u, jnp.zeros((S // 2, 256 - DF), jnp.uint32)], axis=1)
        for m in range(N1 // 2):
            for hf in range(2):
                wp_s[c, m, hf * 128:(hf + 1) * 128, :] = wn_s[hf, pl.ds(m, N2, stride=N1 // 2), :].T

    def smid(m, par):
        k1 = 2 * m + par
        p1 = _dot(t_s[k1, 0:FP, :], m_v[k1, 0])
        p2 = _dot(t_s[k1, TB:TB + FP, :], m_v[k1, 1])
        p3 = _dot(t_s[k1, 2 * TB:2 * TB + FP, :], m_v[k1, 2])
        xr = p1 - p3
        xi = p1 + p2

        def filt(c):
            u = jnp.concatenate(
                [wp_s[c, m, pl.ds(f0, n, stride=8), :]
                 for f0, n in ((1, 28), (7, 28), (2, 28), (6, 28), (3, 28), (5, 28), (0, 29), (4, 28))]
                + [jnp.zeros((7, N2), jnp.uint32)], axis=0)
            u = (u << 16) if par == 0 else (u & jnp.uint32(0xFFFF0000))
            return pltpu.bitcast(u, F32)
        wr, wi = filt(0), filt(1)
        yr = xr * wr - xi * wi
        yi = xr * wi + xi * wr
        q1 = _dot((yr + yi).astype(BF16), m_v[k1, 3])
        q2 = _dot(yi.astype(BF16), m_v[k1, 4])
        q3 = _dot(yr.astype(BF16), m_v[k1, 5])
        a_s[k1, 0:FP, :] = q1 + q2
        a_s[k1, FP:2 * FP, :] = q1 - q3

    NCH = FP // 8

    def dft_chunks(first, n, fwd):
        for j in range(n):
            r = jnp.minimum(first + j, NCH - 1)
            if fwd:
                _dft16_chunk(a_s, f_s, t_s, r, -1, _rows_same)
            else:
                _dft16_chunk(a_s, f_s, z_s, r, +1, _rows_class)

    c_gt.wait()
    c_x[0].wait()
    dfwd(0)
    c_wq.wait()
    wt_s[0, 0:D, :] = w_v[:, 0:D].T
    proj(0, 0)
    c_x[1].wait()
    c_x[2].wait()
    proj(1, 0)
    dfwd(1)
    proj(2, 0)
    c_x[3].wait()
    c_wkv.wait()
    c_gate.wait()
    for c in [c_wo, c_wr, c_wi, c_m, c_git]:
        c.start()
    wt_s[1, 0:D, :] = w_v[:, D:2 * D].T
    wt_s[2, 0:D, :] = w_v[:, 2 * D:3 * D].T
    grow = lax.broadcasted_iota(jnp.int32, (16, D), 0)
    wt_s[2, D:D + 16, :] = jnp.where(grow == 0, jnp.broadcast_to(gate_v[...].reshape(1, D).astype(F32), (16, D)),
                                     0.0).astype(BF16)
    proj(3, 0)
    for i in range(NQ):
        proj(i, 1)
    proj(0, 2)
    proj(1, 2)
    c_wo.wait()
    wot_s[...] = _pad_heads(wo_v[...].T)
    proj(2, 2)
    proj(3, 2)
    dfwd(2)
    dfwd(3)

    prod = (jnp.max(stats["q"], axis=1, keepdims=True) * jnp.max(stats["k"], axis=1, keepdims=True))
    prod = jnp.broadcast_to(prod, (D, 128))
    hr = lax.broadcasted_iota(jnp.int32, (D, 128), 0)
    hc = lax.broadcasted_iota(jnp.int32, (D, 128), 1) * DH
    hsel = (hr >= hc) & (hr < hc + DH)
    bound = jnp.max(jnp.sum(jnp.where(hsel, prod, 0.0), axis=0, keepdims=True))
    vtop = jnp.max(stats["v"])
    safe = (bound <= SAFE_LOG2) & (vtop <= 2.0 ** 40) & (vtop >= 2.0 ** -40)
    c_wr.wait()
    c_wi.wait()
    c_m.wait()
    c_git.wait()

    def head_weights(g, j, q0, tq):
        t0 = q0 // N2
        r0 = g * 112 if isinstance(g, int) else pl.multiple_of(g * 112, 16)
        qg = jnp.concatenate([qt_s[t0 + tt, pl.ds(r0, 112), :] for tt in range(tq // N2)], axis=1)
        w_all = pltpu.bitcast(jnp.concatenate([qg, jnp.zeros((16, tq), BF16)], axis=0), jnp.uint32)
        rows = lax.broadcasted_iota(jnp.int32, (64, tq), 0)
        msk = (rows >= 14 * j) & (rows < 14 * j + 14)
        return pltpu.bitcast(jnp.where(msk, w_all, jnp.uint32(0)), BF16)

    def vrows(h0):
        return jnp.concatenate([vt_s[t, pl.ds(h0, 32), :] for t in range(N1)], axis=1)

    def mo(x, m):
        return x if isinstance(x, int) else pl.multiple_of(x, m)

    def attn_block(g, j0, nh, q0, ta):
        gq = g_s[:, pl.ds(q0, ta)]
        kg = k_s[g]
        for jj in range(nh):
            j = j0 + jj
            p = jnp.exp2(_dot(kg, head_weights(g, j, q0, ta))).astype(BF16)
            h0 = mo((g * 4 + j) * 32, 32)
            acc = _dot(vrows(h0), p)
            ob = (acc * (gq / acc[28:29, :])).astype(BF16)
            for tt in range(ta // N2):
                ot_s[q0 // N2 + tt, pl.ds(h0, 32), :] = ob[:, tt * N2:(tt + 1) * N2]

    per = -(-NCH // 2)

    def body_a(it, carry):
        wperm(it)
        dft_chunks(it * per, per, True)
        attn_block(0, 0, 4, mo(it * 1024, 1024), 1024)
        return carry

    def body_b(it, carry):
        smid(it * 2, 0)
        smid(it * 2, 1)
        attn_block(1 + it // 2, (it % 2) * 2, 2, 0, S)
        smid(it * 2 + 1, 0)
        smid(it * 2 + 1, 1)
        return carry

    def body_c():
        dft_chunks(0, NCH, False)
        attn_block(3, 0, 4, 0, 1024)
        attn_block(3, 0, 4, 1024, 1024)

    def slow_unit(it, carry):
        tq = 128
        h = it // (S // tq)
        q0 = pl.multiple_of((it % (S // tq)) * tq, tq)
        g = h // 4
        s = _dot(k_s[g], head_weights(g, h % 4, q0, tq))
        p = jnp.exp2(s - jnp.max(s, axis=0, keepdims=True)).astype(BF16)
        h0 = pl.multiple_of(h * 32, 32)
        acc = _dot(vrows(h0), p)
        ot_s[q0 // N2, pl.ds(h0, 32), :] = (acc * (g_s[:, pl.ds(q0, tq)] / acc[28:29, :])).astype(BF16)
        return carry

    def loop(n, f):
        def b(i, c):
            f(i)
            return c
        lax.fori_loop(0, n, b, 0)

    @pl.when(safe)
    def _():
        lax.fori_loop(0, 2, body_a, 0)
        lax.fori_loop(0, 4, body_b, 0)
        body_c()

    @pl.when(jnp.logical_not(safe))
    def _():
        loop(2, wperm)
        loop(NCH, lambda r: _dft16_chunk(a_s, f_s, t_s, r, -1, _rows_same))
        loop(N1 // 2, lambda m: (smid(m, 0), smid(m, 1)))
        loop(NCH, lambda r: _dft16_chunk(a_s, f_s, z_s, r, +1, _rows_class))
        lax.fori_loop(0, H * (S // 128), slow_unit, 0)

    chunks = [(0, 512), (512, 512), (1024, 512), (1536, 384), (1920, 128)]

    def out_mm(c0, n):
        sl = slice(c0, c0 + n)
        at = _dot(wot_s[...], jnp.concatenate([ot_s[t] for t in range(c0 // N2, (c0 + n) // N2)], axis=1))

        def zblk(r, m):
            return jnp.concatenate(
                [z_s[t, r:r + m, :] for t in range(c0 // N2, (c0 + n) // N2)], axis=1)
        rr = _dot(git_v[0:112, :], zblk(0, 128))
        gs = [_dot(git_v[112 * r:112 * (r + 1), 0:112], zblk(16 + 112 * r, 112)) for r in (1, 2, 3)]
        return at, rr, gs

    def out_fin(i, c0, n, at, rr, gs):
        sl = slice(c0, c0 + n)
        (g1, h1), (g2, h2), (g3, h3) = ((q[0:CB], q[CB:2 * CB]) for q in gs)
        ev, od = rr[0:CB] + rr[CB:2 * CB], rr[0:CB] - rr[CB:2 * CB]
        ep, em, om, op = ev + g2, ev - g2, od - h2, od + h2
        u, v = g1 + g3, h1 - h3
        dg, sh = g1 - g3, h1 + h3
        a1 = (dg - sh) * RSQRT2
        a3 = (dg + sh) * RSQRT2
        bt = jnp.concatenate([ep + u, om + a1, em - v, op - a3, ep - u, om - a1, em + v, op + a3], axis=0)
        g = g_s[:, sl]
        o_v[:, sl] = (at + (1.0 - g) * bt).astype(BF16)
        c = cp(13 + i, o_v.at[:, sl], o_hbm.at[:, sl])
        c.start()
        return c

    outs = []
    pend = out_mm(*chunks[0])
    for i, (c0, n) in enumerate(chunks):
        nxt = out_mm(*chunks[i + 1]) if i + 1 < len(chunks) else None
        outs.append(out_fin(i, c0, n, *pend))
        pend = nxt
    for c in outs:
        c.wait()


@jax.jit
def pallas_gated_mix__softmax_full_mha__spectral_gfnet__prompt_kernel(
    A_x, A_wqkv, A_wo, B_x, B_w_r, B_w_i, gate_w):
    del B_x
    xt = A_x.reshape(S, D).T
    gt, git, m = _consts()
    gt = jnp.asarray(gt, BF16)
    git = jnp.asarray(git, BF16)
    m = jnp.asarray(m, BF16)
    any_spec = pl.BlockSpec(memory_space=pl.ANY)
    out = pl.pallas_call(
        _kernel,
        out_shape=jax.ShapeDtypeStruct((D, S), BF16),
        in_specs=[any_spec] * 9,
        out_specs=any_spec,
        scratch_shapes=[
            pltpu.VMEM((D, S), BF16),
            pltpu.VMEM((D, 3 * D), BF16),
            pltpu.VMEM((D, D), BF16),
            pltpu.VMEM((2, DF, S), BF16),
            pltpu.VMEM((D,), BF16),
            pltpu.VMEM((464, 2 * CB), BF16),
            pltpu.VMEM((448, 128), BF16),
            pltpu.VMEM((N1, 6, N2, N2), BF16),
            pltpu.VMEM((D, S), BF16),
            pltpu.SemaphoreType.DMA((20,)),
            pltpu.VMEM((4, S, 128), BF16),
            pltpu.VMEM((N1, D, N2), BF16),
            pltpu.VMEM((N1, 512, N2), BF16),
            pltpu.VMEM((N1, 512, N2), BF16),
            pltpu.VMEM((N1, 2 * FP, N2), F32),
            pltpu.VMEM((N1, 3 * TB, N2), BF16),
            pltpu.VMEM((N1, 2 * FP, N2), BF16),
            pltpu.VMEM((1, S), F32),
            pltpu.VMEM((2, S // 2 + 8, 128), jnp.uint32),
            pltpu.VMEM((2, N1 // 2, 256, N2), jnp.uint32),
            pltpu.VMEM((D, 512), BF16),
            pltpu.VMEM((3, D + 16, D), BF16),
            pltpu.VMEM((N1, 2 * FP, N2), F32),
        ],
        compiler_params=pltpu.CompilerParams(vmem_limit_bytes=100 * 1024 * 1024),
    )(xt, A_wqkv, A_wo, B_w_r.T, B_w_i.T, gate_w, gt, git, m)
    return out.T.reshape(1, S, D)
```
